```python
import os as _os
_os.environ.setdefault("JAX_PLATFORMS", "cpu")
import jax
import jax.numpy as jnp

def _softmax(x, axis=-1):
    return jax.nn.softmax(x, axis=axis)
def _gelu(x):
    return jax.nn.gelu(x, approximate=True)
def _silu(x):
    return jax.nn.silu(x)
def _sigmoid(x):
    return jax.nn.sigmoid(x)
def _layernorm(x, axis=-1, eps=1e-5):
    m = jnp.mean(x, axis=axis, keepdims=True)
    v = jnp.var(x, axis=axis, keepdims=True)
    return (x - m) / jnp.sqrt(v + eps)
def _scatter_add(tgt, idx, src, axis=0):
    return tgt.at[idx].add(src)
def _segment_sum(src, seg, n):
    return jax.ops.segment_sum(src, seg, n)
class _Rng:
    def __init__(self, key):
        self._k = key
    def _next(self):
        self._k, sub = jax.random.split(self._k)
        return sub
    def normal(self, shape):
        return jax.random.normal(self._next(), shape, dtype=jnp.bfloat16)
    def randint(self, lo, hi, shape):
        return jax.random.randint(self._next(), shape, lo, hi, dtype=jnp.int32)
    def uniform(self, shape, lo=0.0, hi=1.0):
        return jax.random.uniform(self._next(), shape, jnp.bfloat16, lo, hi)
    def permutation(self, n):
        return jax.random.permutation(self._next(), n)


kernel_name = 'recurrent_scan__sliding_block__dense_activation_mish__prompt'

def setup_inputs():
    _rng = _Rng(jax.random.key(int.from_bytes(__import__("os").urandom(4), "little")))
    _w = (lambda a: (lambda t: t.astype(jnp.bfloat16) if jnp.issubdtype(t.dtype, jnp.floating) else t)(jnp.asarray(a)))
    def _A_setup():
        B, S, D = 1, 2048, 576
        return {
            "x": _w((lambda *s: _rng.normal(s) * 0.05)(B, S, D)),
            "wqkv": _w((lambda *s: _rng.normal(s) * 0.1)(D, 3 * D)),
            "wo": _w((lambda *s: _rng.normal(s) * 0.1)(D, D)),
        }
    _A_in = _A_setup()

    def _B_setup():
        B, S, D, F = 1, 2048, 576, 4608
        return {
            "x": _w((lambda *s: _rng.normal(s) * 0.05)(B, S, D)),
            "w1": _w((lambda *s: _rng.normal(s) * 0.05)(D, F) * (D ** -0.5)),
            "b1": _w((lambda *s: _rng.normal(s) * 0.05)(F)),
            "w2": _w((lambda *s: _rng.normal(s) * 0.05)(F, D) * (F ** -0.5)),
        }
    _B_in = _B_setup()

    return {
        "A_x": _A_in["x"],
        "A_wqkv": _A_in["wqkv"],
        "A_wo": _A_in["wo"],
        "B_x": _B_in["x"],
        "B_w1": _B_in["w1"],
        "B_b1": _B_in["b1"],
        "B_w2": _B_in["w2"],
    }

def reference(A_x, A_wqkv, A_wo, B_x, B_w1, B_b1, B_w2):
    def _A_ref(x, wqkv, wo):
        B, S, D = x.shape
        H = 32; Dh = D // H; W = 256
        qkv = (lambda x, *d: x.transpose(*d))((x @ wqkv).reshape(B, S, 3, H, Dh), 2, 0, 3, 1, 4)
        q, k, v = qkv[0], qkv[1], qkv[2]
        scores = jnp.einsum("bhqd,bhkd->bhqk", q, k) * (Dh ** -0.5)
        idx = jnp.arange(S)
        mask = (idx[:, None] - idx[None, :] >= 0) & (idx[:, None] - idx[None, :] < W)
        scores = jnp.where(mask[None, None], scores, -1e9)
        p = _softmax(scores, axis=-1)
        o = jnp.einsum("bhqk,bhkd->bhqd", p, v)
        return (lambda x, *d: x.transpose(*d))(o, 0, 2, 1, 3).reshape(B, S, D) @ wo

    def _B_ref(x, w1, b1, w2):
        h = jnp.einsum("bsd,df->bsf", x, w1) + b1
        sp = jnp.log1p(jnp.exp(-jnp.abs(h))) + jnp.where(h > 0, h, jnp.zeros_like(h))
        act = h * jnp.tanh(sp)
        return jnp.einsum("bsf,fd->bsd", act, w2)

    x = A_x
    xn = _layernorm(x, axis=-1)
    s = _A_ref(xn, A_wqkv, A_wo)
    g = _silu(_B_ref(xn, B_w1, B_b1, B_w2))
    return x + s * g
```

```python
import jax
import jax.numpy as jnp
from jax import lax
import jax.experimental.pallas as pl
import jax.experimental.pallas.tpu as pltpu

S, D, F = 2048, 576, 4608
H, DH, W = 32, 18, 256
TQ = 512
T = 256
G = 4
FC = F // G
PAD = 384
L1, L2, L3 = 8, 8, 3
LOG2E = 1.4426950408889634
NEG = -1e9 * LOG2E
BF = jnp.bfloat16
F32 = jnp.float32
NT = (((1,), (1,)), ((), ()))


def _layernorm(t0, x_ref, xn_ref):
    x = x_ref[:, pl.ds(t0, TQ)].astype(F32)
    mu = jnp.mean(x, axis=0, keepdims=True)
    xc = x - mu
    var = jnp.mean(xc * xc, axis=0, keepdims=True)
    xnt = xc * lax.rsqrt(var + 1e-5)
    xnt = xnt.astype(BF)
    rows = pl.ds(t0, TQ)
    for t in range(4):
        xn_ref[rows, 128 * t:128 * t + 128] = xnt[128 * t:128 * t + 128].T
    xn_ref[rows, 512:576] = jnp.concatenate([xnt[512:576]] * 2, axis=0).T[:, 0:64]


def _project(t0, wqkv_ref, wvt_ref, xn_ref, q_ref, k_ref, vt_ref):
    rows = pl.ds(t0, TQ)
    krows = pl.ds(PAD + t0, TQ)

    def proj(lo, up):
        return jnp.dot(xn_ref[rows, :], wqkv_ref[:, lo:up], preferred_element_type=F32)

    q = proj(0, 640)
    k2 = proj(640, 1152)
    vt_ref[:, krows] = lax.dot_general(
        wvt_ref[...], xn_ref[rows, :], NT, preferred_element_type=F32).astype(BF)
    hi = lax.broadcasted_iota(jnp.int32, (TQ, 128), 1) >= 64
    qr = [pltpu.roll(q[:, 128 * t:128 * t + 128] * (DH ** -0.5 * LOG2E), 64, 1) for t in range(5)]
    qs = [qr[0]] + [jnp.where(hi, qr[t], qr[t - 1]) for t in range(1, 5)] + qr[:4]
    for t in range(9):
        q_ref[t, rows, :] = qs[t].astype(BF)
    kt = [q[:, 512:640]] + [k2[:, 128 * t:128 * t + 128] for t in range(4)]
    for t in range(5):
        k_ref[t, krows, :] = kt[t].astype(BF)
        if t:
            k_ref[4 + t, krows, :] = jnp.where(hi, kt[t - 1], kt[t]).astype(BF)


def _attention(g, t0, q_ref, k_ref, vt_ref, bias_ref, ot_ref):
    l64 = lax.broadcasted_iota(jnp.int32, (64, 128), 1)
    lo = lax.broadcasted_iota(jnp.int32, (40, 128), 1) < 64
    row40 = lax.broadcasted_iota(jnp.int32, (40, 128), 0)
    row8 = lax.broadcasted_iota(jnp.int32, (8, 128), 0)

    def qk(j, b):
        c0 = 64 + 144 * g + 36 * j
        tile = c0 >> 7
        tile = jnp.where(((c0 + 35) >> 7) != tile, tile + 5, tile)
        q = q_ref[tile, pl.ds(pl.multiple_of(t0 + 64 * b, 64), 64), :].astype(F32)
        qa = jnp.where(((l64 - c0) & 127) < DH, q, 0.0).astype(BF)
        qb = jnp.where(((l64 - c0 - DH) & 127) < DH, q, 0.0).astype(BF)
        qbd = jnp.concatenate([qa, qb] if b % 2 == 0 else [qb, qa], axis=0)
        kw = k_ref[tile, pl.ds(pl.multiple_of(t0 + 64 * b + PAD - W, 64), 320), :]
        return lax.dot_general(kw, qbd, NT, preferred_element_type=F32)

    def softmax(s, b):
        s = s + bias_ref[b]
        e = jnp.exp2(s - jnp.max(s, axis=0, keepdims=True))
        return e.astype(BF), 1.0 / jnp.sum(e, axis=0, keepdims=True)

    def pv(j, b, pt, rl):
        w0 = (36 * j) // 16 * 16
        vrows = pl.ds(pl.multiple_of(144 * g + w0, 16), 48)
        if b % 2 == 0:
            vw = vt_ref[vrows, pl.ds(pl.multiple_of(t0 + 64 * b + PAD - W, 128), 320)]
        else:
            vw = vt_ref[vrows, pl.ds(pl.multiple_of(t0 + 64 * b + PAD - W - 64, 128), 384)]
            pt = jnp.concatenate([jnp.zeros((64, 128), BF), pt], axis=0)
        o = jnp.dot(vw, pt, preferred_element_type=F32)
        d8 = (36 * j) // 8 * 8 - w0
        return o[d8:d8 + 40] * rl

    def pair(j, c):
        oe, oo = res.pop((j, 2 * c)), res.pop((j, 2 * c + 1))
        a = jnp.where(lo, oe, oo)
        bm = pltpu.roll(jnp.where(lo, oo, oe), 64, 1)
        return jnp.where(row40 < (36 * j) % 8 + DH, a, bm)

    def emit(c):
        rows = []
        for j in range(2):
            e_, o_ = pair(2 * j, c), pair(2 * j + 1, c)
            rows += [e_[0:32], jnp.where(row8 < 4, e_[32:40], o_[0:8]), o_[8:40]]
        ot_ref[pl.ds(pl.multiple_of(144 * g, 16), 144), 128 * c:128 * c + 128] = (
            jnp.concatenate(rows, axis=0).astype(BF))

    units = [(j, 2 * c + e) for c in range(T // 128) for j in range(4) for e in range(2)]
    n, sc, pr, res = len(units), {}, {}, {}
    for it in range(n + L1 + L2 + L3):
        if it < n:
            sc[it] = qk(*units[it])
        u = it - L1
        if 0 <= u < n:
            pr[u] = softmax(sc.pop(u), units[u][1])
        u -= L2
        if 0 <= u < n:
            res[units[u]] = pv(*units[u], *pr.pop(u))
        u -= L3
        if 0 <= u < n and u % 8 == 7:
            emit(units[u][1] // 2)
        yield


def _ffn(g, xn_ref, t0, w1_ref, b1_ref, w2t_ref, acc_ref, nsub=3):
    w = FC // nsub
    for c in range(nsub):
        cs = pl.ds(pl.multiple_of(g * FC + c * w, 128), w)
        h = jnp.dot(xn_ref[pl.ds(t0, T), :], w1_ref[:, cs], preferred_element_type=F32)
        yield
        h = h + b1_ref[:, cs].astype(F32)
        n = jnp.exp2(jnp.minimum(h, 20.0) * LOG2E)
        u = n * (n + 2.0)
        act = (h * u * pl.reciprocal(u + 2.0, approx=True)).astype(BF)
        yield
        acc_ref[...] += lax.dot_general(w2t_ref[:, cs], act, NT, preferred_element_type=F32)
        yield


def _transpose(src_ref, col0, dst_ref):
    for j in range(5):
        r = slice(128 * j, 128 * j + 128) if j < 4 else slice(D - 128, D)
        for t in range(5):
            c = 128 * t if t < 4 else D - 128
            dst_ref[c:c + 128, r] = src_ref[r, col0 + c:col0 + c + 128].T


def _kernel(x_hbm, wqkv_hbm, wo_hbm, w1_hbm, b1_ref, w2t_hbm, o_ref,
            x_ref, wqkv_ref, wo_ref, w1_ref, w2t_ref, wot_ref, wvt_ref,
            xn_ref, q_ref, k_ref, vt_ref, ot_ref, acc_ref, bias_ref, sem):
    i = pl.program_id(0)

    @pl.when(i == 0)
    def _():
        cp_x0 = pltpu.make_async_copy(x_hbm.at[:, 0:TQ], x_ref.at[:, 0:TQ], sem.at[0])
        cp_x1 = pltpu.make_async_copy(x_hbm.at[:, TQ:S], x_ref.at[:, TQ:S], sem.at[1])
        cp_qkv = pltpu.make_async_copy(wqkv_hbm, wqkv_ref, sem.at[2])
        cp_wo = pltpu.make_async_copy(wo_hbm, wo_ref, sem.at[3])
        cp_w1 = pltpu.make_async_copy(w1_hbm, w1_ref, sem.at[4])
        cp_w2 = pltpu.make_async_copy(w2t_hbm, w2t_ref, sem.at[5])
        for cp in (cp_qkv, cp_x0, cp_x1, cp_wo, cp_w1, cp_w2):
            cp.start()
        k_ref[:, 0:PAD, :] = jnp.zeros((9, PAD, 128), BF)
        vt_ref[:, 0:PAD] = jnp.zeros((D, PAD), BF)
        cp_x0.wait()
        cp_qkv.wait()
        _transpose(wqkv_ref, 2 * D, wvt_ref)
        cp_x1.wait()

        @pl.loop(0, S // TQ)
        def _(c):
            _layernorm(pl.multiple_of(c * TQ, TQ), x_ref, xn_ref)

        @pl.loop(0, S // TQ)
        def _(c):
            _project(pl.multiple_of(c * TQ, TQ), wqkv_ref, wvt_ref, xn_ref, q_ref, k_ref, vt_ref)

        cp_wo.wait()
        _transpose(wo_ref, 0, wot_ref)
        cp_w1.wait()
        cp_w2.wait()

    t0 = pl.multiple_of(i * T, T)

    @pl.when(i <= 1)
    def _():
        r = lax.broadcasted_iota(jnp.int32, (320, 128), 0)
        qi = lax.broadcasted_iota(jnp.int32, (320, 128), 1) & 63
        for b in range(T // 64):
            ok = (r > qi) & (r <= qi + W) & (r >= W - t0 - 64 * b)
            bias_ref[b] = jnp.where(ok, 0.0, NEG)

    acc_ref[...] = jnp.zeros_like(acc_ref)

    @pl.loop(0, G)
    def _(g):
        att = _attention(g, t0, q_ref, k_ref, vt_ref, bias_ref, ot_ref)
        ffn = _ffn(g, xn_ref, t0, w1_ref, b1_ref, w2t_ref, acc_ref)
        for step, _ in enumerate(att):
            if step % 3 == 0:
                next(ffn, None)
        for _ in ffn:
            pass

    gt = acc_ref[...]
    st = jnp.dot(wot_ref[...], ot_ref[...], preferred_element_type=F32)
    y = st * gt * (1.0 / (1.0 + jnp.exp(-gt)))
    o_ref[...] = (x_ref[:, pl.ds(t0, T)].astype(F32) + y).astype(o_ref.dtype)


@jax.jit
def pallas_recurrent_scan__sliding_block__dense_activation_mish__prompt_kernel(
    A_x, A_wqkv, A_wo, B_x, B_w1, B_b1, B_w2,
):
    del B_x
    any_spec = pl.BlockSpec(memory_space=pl.ANY)
    out = pl.pallas_call(
        _kernel,
        grid=(S // T,),
        in_specs=[any_spec, any_spec, any_spec, any_spec,
                  pl.BlockSpec((1, F), lambda i: (0, 0)), any_spec],
        out_specs=pl.BlockSpec((D, T), lambda i: (0, i)),
        out_shape=jax.ShapeDtypeStruct((D, S), A_x.dtype),
        scratch_shapes=[
            pltpu.VMEM((D, S), BF),
            pltpu.VMEM((D, 3 * D), BF), pltpu.VMEM((D, D), BF), pltpu.VMEM((D, F), BF),
            pltpu.VMEM((D, F), BF), pltpu.VMEM((D, D), BF), pltpu.VMEM((D, D), BF),
            pltpu.VMEM((S, D), BF), pltpu.VMEM((9, S, 128), BF),
            pltpu.VMEM((9, PAD + S, 128), BF), pltpu.VMEM((D, PAD + S), BF),
            pltpu.VMEM((D, T), BF), pltpu.VMEM((D, T), F32),
            pltpu.VMEM((T // 64, 320, 128), F32),
            pltpu.SemaphoreType.DMA((6,)),
        ],
        compiler_params=pltpu.CompilerParams(
            dimension_semantics=("arbitrary",), vmem_limit_bytes=100 * 1024 * 1024),
        name="fused_block",
    )(A_x.reshape(S, D).T, A_wqkv, A_wo, B_w1, B_b1.reshape(1, F), B_w2.T)
    return out.T.reshape(1, S, D)
```
